```python
import os as _os
_os.environ.setdefault("JAX_PLATFORMS", "cpu")
import jax
import jax.numpy as jnp

def _softmax(x, axis=-1):
    return jax.nn.softmax(x, axis=axis)
def _gelu(x):
    return jax.nn.gelu(x, approximate=True)
def _silu(x):
    return jax.nn.silu(x)
def _sigmoid(x):
    return jax.nn.sigmoid(x)
def _layernorm(x, axis=-1, eps=1e-5):
    m = jnp.mean(x, axis=axis, keepdims=True)
    v = jnp.var(x, axis=axis, keepdims=True)
    return (x - m) / jnp.sqrt(v + eps)
def _scatter_add(tgt, idx, src, axis=0):
    return tgt.at[idx].add(src)
def _segment_sum(src, seg, n):
    return jax.ops.segment_sum(src, seg, n)
class _Rng:
    def __init__(self, key):
        self._k = key
    def _next(self):
        self._k, sub = jax.random.split(self._k)
        return sub
    def normal(self, shape):
        return jax.random.normal(self._next(), shape, dtype=jnp.bfloat16)
    def randint(self, lo, hi, shape):
        return jax.random.randint(self._next(), shape, lo, hi, dtype=jnp.int32)
    def uniform(self, shape, lo=0.0, hi=1.0):
        return jax.random.uniform(self._next(), shape, jnp.bfloat16, lo, hi)
    def permutation(self, n):
        return jax.random.permutation(self._next(), n)


kernel_name = 'recurrent_scan__grouped_kv_mqa__mixer_s_mlp__prompt'

def setup_inputs():
    _rng = _Rng(jax.random.key(int.from_bytes(__import__("os").urandom(4), "little")))
    _w = (lambda a: (lambda t: t.astype(jnp.bfloat16) if jnp.issubdtype(t.dtype, jnp.floating) else t)(jnp.asarray(a)))
    def _A_setup():
        B, S, D, H = 1, 2048, 512, 32
        Dh = D // H
        return {
            "x": _w((lambda *s: _rng.normal(s) * 0.05)(B, S, D)),
            "wq": _w((lambda *s: _rng.normal(s) * 0.05)(D, H * Dh)),
            "wk": _w((lambda *s: _rng.normal(s) * 0.05)(D, Dh)),
            "wv": _w((lambda *s: _rng.normal(s) * 0.05)(D, Dh)),
            "wo": _w((lambda *s: _rng.normal(s) * 0.05)(H * Dh, D)),
        }
    _A_in = _A_setup()

    def _B_setup():
        B, S, D, F = 1, 2048, 512, 1792
        return {
            "x":  _w((lambda *s: _rng.normal(s) * 0.05)(B, S, D)),
            "w1": _w((lambda *s: _rng.normal(s) * 0.8)(D, D) * (D ** -0.5)),
            "w2": _w((lambda *s: _rng.normal(s) * 0.8)(D, D) * (D ** -0.5)),
            "w3": _w((lambda *s: _rng.normal(s) * 0.8)(D, F) * (D ** -0.5)),
            "w4": _w((lambda *s: _rng.normal(s) * 0.8)(F, D) * (F ** -0.5)),
        }
    _B_in = _B_setup()

    return {
        "A_x": _A_in["x"],
        "A_wq": _A_in["wq"],
        "A_wk": _A_in["wk"],
        "A_wv": _A_in["wv"],
        "A_wo": _A_in["wo"],
        "B_x": _B_in["x"],
        "B_w1": _B_in["w1"],
        "B_w2": _B_in["w2"],
        "B_w3": _B_in["w3"],
        "B_w4": _B_in["w4"],
    }

def reference(A_x, A_wq, A_wk, A_wv, A_wo, B_x, B_w1, B_w2, B_w3, B_w4):
    def _A_ref(x, wq, wk, wv, wo):
        B, S, D = x.shape
        H = 32
        Dh = D // H
        q = (lambda x, *d: x.transpose(*d))((x @ wq).reshape(B, S, H, Dh), 0, 2, 1, 3)
        k = x @ wk
        v = x @ wv
        scores = jnp.einsum("bhqd,bkd->bhqk", q, k) * (Dh ** -0.5)
        p = _softmax(scores, axis=-1)
        o = jnp.einsum("bhqk,bkd->bhqd", p, v)
        return (lambda x, *d: x.transpose(*d))(o, 0, 2, 1, 3).reshape(B, S, H * Dh) @ wo

    def _B_ref(x, w1, w2, w3, w4):
        B, S, D = x.shape
        h = _gelu(_layernorm(x, axis=-1) @ w1)
        c = D // 4
        g0 = jnp.pad(h[:, :, 0*c:1*c], ((0, 0), (1, 0), (0, 0)))[:, :S, :]
        g1 = jnp.pad(h[:, :, 1*c:2*c], ((0, 0), (0, 1), (0, 0)))[:, 1:, :]
        g2 = jnp.pad(h[:, :, 2*c:3*c], ((0, 0), (2, 0), (0, 0)))[:, :S, :]
        g3 = jnp.pad(h[:, :, 3*c:   ], ((0, 0), (0, 2), (0, 0)))[:, 2:, :]
        hs = jnp.concatenate([g0, g1, g2, g3], axis=-1) @ w2
        x1 = x + hs
        h2 = _gelu(_layernorm(x1, axis=-1) @ w3) @ w4
        return x1 + h2

    x = A_x
    xn = _layernorm(x, axis=-1)
    s = _A_ref(xn, A_wq, A_wk, A_wv, A_wo)
    g = _silu(_B_ref(xn, B_w1, B_w2, B_w3, B_w4))
    return x + s * g
```

```python
import functools
import jax
import jax.numpy as jnp
from jax import lax
import jax.experimental.pallas as pl
import jax.experimental.pallas.tpu as pltpu

S, D, H, DH, F = 2048, 512, 32, 16, 1792
LOG2E = 1.4426950408889634
bf16, f32 = jnp.bfloat16, jnp.float32
NT = (((1,), (1,)), ((), ()))
PAD = 16

def _ln(x):
    m = jnp.mean(x, axis=-1, keepdims=True)
    d = x - m
    v = jnp.mean(d * d, axis=-1, keepdims=True)
    return d * lax.rsqrt(v + 1e-5)

def _gelu(x):
    hx = 0.5 * x
    return hx + hx * jnp.tanh(x * (0.7978845608028654 + (0.7978845608028654 * 0.044715) * (x * x)))

def _kernel(x_h, wq_h, wkt_h, wvt_h, wo_h, w1_h, w2_h, w3_h, w4_h, o_ref,
            x_s, xn_s, k_s, vt_s, qt_s, ot_s, sa, sb, m_s, wq_s, wa_s, wo_ref, w1_ref, w2_ref, w3_ref, w4_ref, sems,
            *, tq, ck, lag, dm, un, rep, tm):
    i = pl.program_id(0)
    nb = S // tq
    nc = S // ck
    NP = nb * H
    pairs = [(x_h.at[b * tq:(b + 1) * tq], x_s.at[b * tq:(b + 1) * tq]) for b in range(nb)]
    pairs += [(wq_h, wq_s), (wkt_h, wa_s.at[D:D + DH]), (wvt_h, wa_s.at[D + DH:D + 2 * DH])]
    pairs += [(w1_h, w1_ref), (wo_h, wo_ref), (w2_h, w2_ref), (w3_h, w3_ref), (w4_h, w4_ref)]
    copies = [pltpu.make_async_copy(a, b, sems.at[n]) for n, (a, b) in enumerate(pairs)]

    @pl.when(i == 0)
    def _():
        for n in [nb, 0, nb + 1, nb + 2] + list(range(1, nb)):
            copies[n].start()
        m_s[...] = jnp.zeros((16, tq), f32)
        xn_s[0:PAD, :] = jnp.zeros((PAD, D), bf16)
        xn_s[S + PAD:S + 2 * PAD, :] = jnp.zeros((PAD, D), bf16)
        copies[nb].wait()
        wa_s[0:D, :] = wq_s[...].T
        copies[nb + 1].wait()
        copies[nb + 2].wait()
        for b in range(nb):
            r = b * tq
            copies[b].wait()
            if b == nb - 1:
                for cp in copies[nb + 3:]:
                    cp.start()
            xnb = _ln(x_s[r:r + tq, :].astype(f32)).astype(bf16)
            xn_s[PAD + r:PAD + r + tq, :] = xnb
            a = lax.dot_general(wa_s[...], xnb, NT, preferred_element_type=f32)
            qt_s[b * D:(b + 1) * D, :] = (a[0:D] * (DH ** -0.5 * LOG2E)).astype(bf16)
            k_s[r:r + tq, :] = a[D:D + DH].T.astype(bf16)
            vt_s[:, r:r + tq] = a[D + DH:D + 2 * DH].astype(bf16)

        def qk_chunk(t, c, dst, mx):
            t = jnp.minimum(t, NP - 1)
            q = qt_s[pl.ds(pl.multiple_of(t * DH, DH), DH), :]
            s = jnp.dot(k_s[c * ck:(c + 1) * ck, :], q, preferred_element_type=f32)
            dst[c * ck:(c + 1) * ck, :] = s
            cm = jnp.max(s.reshape(ck // 8, 8, tq), axis=0)
            return cm if mx is None else jnp.maximum(mx, cm)

        def step(t, m8, mx, src, dst, pend):
            m_s[0:8, :] = jnp.broadcast_to(jnp.max(m8, axis=0, keepdims=True), (8, tq))
            z = pl.multiple_of((t // NP) * 8, 8)
            acc = None; l = None; mx2 = None
            for c in range(nc):
                m = m_s[pl.ds(z, 8), :]
                if c + lag < nc:
                    mx = qk_chunk(t + 1, c + lag, dst, mx)
                    pend.append(mx)
                p = jnp.exp2(src[c * ck:(c + 1) * ck, :].reshape(ck // 8, 8, tq) - m[None])
                for g in reversed(range(ck // 16)):
                    cl = p[2 * g] + p[2 * g + 1]
                    l = cl if l is None else l + cl
                o = jnp.dot(vt_s[:, c * ck:(c + 1) * ck], p.reshape(ck, tq).astype(bf16), preferred_element_type=f32)
                acc = o if acc is None else acc + o
                if c + lag >= nc:
                    mx2 = qk_chunk(t + 2, c + lag - nc, src, mx2)
                    pend.append(mx2)
                if len(pend) > dm:
                    m_s[8:16, 0:128] = pend.pop(0)[:, tq - 128:]
            ot_s[pl.ds(pl.multiple_of(t * DH, DH), DH), :] = (acc / jnp.sum(l, axis=0, keepdims=True)).astype(bf16)
            return mx, mx2

        m8 = None; mx = None
        for c in range(nc):
            m8 = qk_chunk(0, c, sa, m8)
        for c in range(lag):
            mx = qk_chunk(1, c, sb, mx)
        def group(j, carry):
            if rep > 1:
                j = j % (NP // un)
            pend = []
            m8, mx = carry
            for u in range(0, un, 2):
                m8, mx = step(un * j + u, m8, mx, sa, sb, pend)
                m8, mx = step(un * j + u + 1, m8, mx, sb, sa, pend)
            return m8, mx
        lax.fori_loop(0, NP // un * rep, group, (m8, mx))
        for cp in copies[nb + 3:]:
            cp.wait()

    r0 = pl.multiple_of(i * tm, tm)
    b = (i * tm) // tq
    ot = ot_s[pl.ds(pl.multiple_of(b * D, D), D), pl.ds(pl.multiple_of((i * tm) % tq, tm), tm)]
    xe = xn_s[pl.ds(r0, tm + 2 * PAD), :].astype(f32)
    h = _gelu(jnp.dot(_ln(xe).astype(bf16), w1_ref[...], preferred_element_type=f32))
    att = lax.dot_general(ot, wo_ref[...], (((0,), (0,)), ((), ())), preferred_element_type=f32)
    c = D // 4
    hsh = jnp.concatenate([h[PAD - s:PAD - s + tm, n * c:(n + 1) * c] for n, s in enumerate((1, -1, 2, -2))],
                          axis=-1).astype(bf16)
    x1 = xe[PAD:PAD + tm] + jnp.dot(hsh, w2_ref[...], preferred_element_type=f32)
    a = _gelu(jnp.dot(_ln(x1).astype(bf16), w3_ref[...], preferred_element_type=f32)).astype(bf16)
    y = x1 + jnp.dot(a, w4_ref[...], preferred_element_type=f32)
    g = y * jax.nn.sigmoid(y)
    o_ref[...] = (x_s[pl.ds(r0, tm), :].astype(f32) + att * g).astype(o_ref.dtype)

def _run(A_x, A_wq, A_wk, A_wv, A_wo, B_x, B_w1, B_w2, B_w3, B_w4, tq=512, ck=128, lag=2, dm=3, un=4, rep=1, tm=512, flags=None):
    x = A_x.reshape(S, D)
    hin = [x, A_wq, A_wk.T, A_wv.T, A_wo, B_w1, B_w2, B_w3, B_w4]
    nb = S // tq
    out = pl.pallas_call(
        functools.partial(_kernel, tq=tq, ck=ck, lag=lag, dm=dm, un=un, rep=rep, tm=tm),
        grid=(S // tm,),
        in_specs=[pl.BlockSpec(memory_space=pl.ANY)] * 9,
        out_specs=pl.BlockSpec((tm, D), lambda i: (i, 0)),
        out_shape=jax.ShapeDtypeStruct((S, D), bf16),
        scratch_shapes=[pltpu.VMEM((S, D), bf16), pltpu.VMEM((S + 2 * PAD, D), bf16), pltpu.VMEM((S, DH), bf16),
                        pltpu.VMEM((DH, S), bf16), pltpu.VMEM((nb * D, tq), bf16), pltpu.VMEM((nb * D, tq), bf16),
                        pltpu.VMEM((S, tq), f32), pltpu.VMEM((S, tq), f32), pltpu.VMEM((16, tq), f32),
                        pltpu.VMEM((D, D), bf16), pltpu.VMEM((D + 2 * DH, D), bf16)]
                       + [pltpu.VMEM(a.shape, bf16) for a in hin[4:]] + [pltpu.SemaphoreType.DMA((nb + 8,))],
        compiler_params=pltpu.CompilerParams(dimension_semantics=("arbitrary",), vmem_limit_bytes=100 * 1024 * 1024, flags=flags),
    )(*hin)
    return out.reshape(1, S, D)


@jax.jit
def pallas_recurrent_scan__grouped_kv_mqa__mixer_s_mlp__prompt_kernel(
        A_x, A_wq, A_wk, A_wv, A_wo, B_x, B_w1, B_w2, B_w3, B_w4):
    return _run(A_x, A_wq, A_wk, A_wv, A_wo, B_x, B_w1, B_w2, B_w3, B_w4, un=8)
```

```python
import functools
import jax
import jax.numpy as jnp
from jax import lax
import jax.experimental.pallas as pl
import jax.experimental.pallas.tpu as pltpu

S, D, H, DH, F = 2048, 512, 32, 16, 1792
LOG2E = 1.4426950408889634
bf16, f32 = jnp.bfloat16, jnp.float32
NT = (((1,), (1,)), ((), ()))
PAD = 16
VK = 16

def _ln(x):
    m = jnp.mean(x, axis=-1, keepdims=True)
    d = x - m
    v = jnp.mean(d * d, axis=-1, keepdims=True)
    return d * lax.rsqrt(v + 1e-5)

def _gelu(x):
    hx = 0.5 * x
    return hx + hx * jnp.tanh(x * (0.7978845608028654 + (0.7978845608028654 * 0.044715) * (x * x)))

def _kernel(x_h, wq_h, wkt_h, wvt_h, wo_h, w1_h, w2_h, w3_h, w4_h, o_ref,
            x_s, xn_s, k_s, vt_s, qt_s, ot_s, sa, sb, m_s, kb_s, qa_s, qb_s, wq_s, wa_s, wo_ref, w1_ref, w2_ref, w3_ref, w4_ref, sems,
            *, tq, ck, lag, dm, un, tm, vpu):
    i = pl.program_id(0)
    nb = S // tq
    nc = S // ck
    NP = nb * H
    pairs = [(x_h.at[b * tq:(b + 1) * tq], x_s.at[b * tq:(b + 1) * tq]) for b in range(nb)]
    pairs += [(wq_h, wq_s), (wkt_h, wa_s.at[D:D + DH]), (wvt_h, wa_s.at[D + DH:D + 2 * DH])]
    pairs += [(w1_h, w1_ref), (wo_h, wo_ref), (w2_h, w2_ref), (w3_h, w3_ref), (w4_h, w4_ref)]
    copies = [pltpu.make_async_copy(a, b, sems.at[n]) for n, (a, b) in enumerate(pairs)]

    @pl.when(i == 0)
    def _():
        for n in [nb, 0, nb + 1, nb + 2] + list(range(1, nb)):
            copies[n].start()
        m_s[...] = jnp.zeros((16, tq), f32)
        xn_s[0:PAD, :] = jnp.zeros((PAD, D), bf16)
        xn_s[S + PAD:S + 2 * PAD, :] = jnp.zeros((PAD, D), bf16)
        copies[nb].wait()
        wa_s[0:D, :] = wq_s[...].T
        copies[nb + 1].wait()
        copies[nb + 2].wait()
        for b in range(nb):
            r = b * tq
            copies[b].wait()
            if b == nb - 1:
                for cp in copies[nb + 3:]:
                    cp.start()
            xnb = _ln(x_s[r:r + tq, :].astype(f32)).astype(bf16)
            xn_s[PAD + r:PAD + r + tq, :] = xnb
            a = lax.dot_general(wa_s[...], xnb, NT, preferred_element_type=f32)
            qt_s[b * D:(b + 1) * D, :] = (a[0:D] * (DH ** -0.5 * LOG2E)).astype(bf16)
            kk = a[D:D + DH].T.astype(bf16)
            k_s[r:r + tq, :] = kk
            for c in range(r // ck, (r + tq) // ck):
                if c in vpu:
                    e = (c + 1) * ck - r
                    kf = kk[e - VK:e].astype(f32)
                    for d in range(DH):
                        kb_s[vpu.index(c), d] = jnp.broadcast_to(kf[:, d:d + 1], (VK, 128))
            vt_s[:, r:r + tq] = a[D + DH:D + 2 * DH].astype(bf16)

        def qk_chunk(t, c, dst, mx, qb=None):
            t = jnp.minimum(t, NP - 1)
            q = qt_s[pl.ds(pl.multiple_of(t * DH, DH), DH), :]
            if qb is None or c not in vpu:
                s = jnp.dot(k_s[c * ck:(c + 1) * ck, :], q, preferred_element_type=f32)
            else:
                s = jnp.dot(k_s[c * ck:(c + 1) * ck - VK, :], q, preferred_element_type=f32)
                s = jnp.concatenate([s, qb.pop(c)], axis=0)
            dst[c * ck:(c + 1) * ck, :] = s
            cm = jnp.max(s.reshape(ck // 8, 8, tq), axis=0)
            return cm if mx is None else jnp.maximum(mx, cm)

        def step(t, m8, mx, src, dst, pend, qb):
            qf = qt_s[pl.ds(pl.multiple_of(jnp.minimum(t + 1, NP - 1) * DH, DH), DH), :].astype(f32)
            for d in range(DH):
                qb[d] = jnp.broadcast_to(qf[d:d + 1], (8, tq))
            m_s[0:8, :] = jnp.broadcast_to(jnp.max(m8, axis=0, keepdims=True), (8, tq))
            z = pl.multiple_of((t // NP) * 8, 8)
            acc = None; l = None; mx2 = None; sv = {}
            for c in range(nc):
                m = m_s[pl.ds(z, 8), :]
                if c + lag < nc:
                    cc = c + lag
                    tg = min([v for v in vpu if v >= cc], default=None)
                    if tg is not None:
                        p0 = max([v for v in vpu if v < cc], default=lag - 1)
                        n, k = tg - p0, cc - p0
                        for d in range((k - 1) * DH // n, k * DH // n):
                            kb = kb_s[pl.ds(vpu.index(tg) + z, 1), d][0]
                            pr = jnp.concatenate([kb] * (tq // 128), axis=1) * jnp.concatenate([qb[d]] * (VK // 8), axis=0)
                            sv[tg] = sv[tg] + pr if tg in sv else pr
                    mx = qk_chunk(t + 1, cc, dst, mx, sv)
                    pend.append(mx)
                p = jnp.exp2(src[c * ck:(c + 1) * ck, :].reshape(ck // 8, 8, tq) - m[None])
                for g in reversed(range(ck // 16)):
                    cl = p[2 * g] + p[2 * g + 1]
                    l = cl if l is None else l + cl
                o = jnp.dot(vt_s[:, c * ck:(c + 1) * ck], p.reshape(ck, tq).astype(bf16), preferred_element_type=f32)
                acc = o if acc is None else acc + o
                if c + lag >= nc:
                    mx2 = qk_chunk(t + 2, c + lag - nc, src, mx2)
                    pend.append(mx2)
                if len(pend) > dm:
                    pm = pend.pop(0)[:, tq - 128:]
                    m_s[8:16, 0:128] = pm
                    kb_s[len(vpu), 0, 0:8, :] = pm
            ot_s[pl.ds(pl.multiple_of(t * DH, DH), DH), :] = (acc / jnp.sum(l, axis=0, keepdims=True)).astype(bf16)
            return mx, mx2

        m8 = None; mx = None
        for c in range(nc):
            m8 = qk_chunk(0, c, sa, m8)
        for c in range(lag):
            mx = qk_chunk(1, c, sb, mx)
        def group(j, carry):
            pend = []
            m8, mx = carry
            for u in range(0, un, 2):
                m8, mx = step(un * j + u, m8, mx, sa, sb, pend, qa_s)
                m8, mx = step(un * j + u + 1, m8, mx, sb, sa, pend, qb_s)
            return m8, mx
        lax.fori_loop(0, NP // un, group, (m8, mx))
        for cp in copies[nb + 3:]:
            cp.wait()

    r0 = pl.multiple_of(i * tm, tm)
    b = (i * tm) // tq
    ot = ot_s[pl.ds(pl.multiple_of(b * D, D), D), pl.ds(pl.multiple_of((i * tm) % tq, tm), tm)]
    xe = xn_s[pl.ds(r0, tm + 2 * PAD), :].astype(f32)
    h = _gelu(jnp.dot(_ln(xe).astype(bf16), w1_ref[...], preferred_element_type=f32))
    att = lax.dot_general(ot, wo_ref[...], (((0,), (0,)), ((), ())), preferred_element_type=f32)
    c = D // 4
    hsh = jnp.concatenate([h[PAD - s:PAD - s + tm, n * c:(n + 1) * c] for n, s in enumerate((1, -1, 2, -2))],
                          axis=-1).astype(bf16)
    x1 = xe[PAD:PAD + tm] + jnp.dot(hsh, w2_ref[...], preferred_element_type=f32)
    a = _gelu(jnp.dot(_ln(x1).astype(bf16), w3_ref[...], preferred_element_type=f32)).astype(bf16)
    y = x1 + jnp.dot(a, w4_ref[...], preferred_element_type=f32)
    g = y * jax.nn.sigmoid(y)
    o_ref[...] = (x_s[pl.ds(r0, tm), :].astype(f32) + att * g).astype(o_ref.dtype)

def _run(A_x, A_wq, A_wk, A_wv, A_wo, B_x, B_w1, B_w2, B_w3, B_w4, tq=512, ck=128, lag=1, dm=2, un=8, tm=512, nv=5):
    vpu = tuple(lag - 1 + ((n + 1) * (16 - lag)) // nv for n in range(nv))
    x = A_x.reshape(S, D)
    hin = [x, A_wq, A_wk.T, A_wv.T, A_wo, B_w1, B_w2, B_w3, B_w4]
    nb = S // tq
    out = pl.pallas_call(
        functools.partial(_kernel, tq=tq, ck=ck, lag=lag, dm=dm, un=un, tm=tm, vpu=vpu),
        grid=(S // tm,),
        in_specs=[pl.BlockSpec(memory_space=pl.ANY)] * 9,
        out_specs=pl.BlockSpec((tm, D), lambda i: (i, 0)),
        out_shape=jax.ShapeDtypeStruct((S, D), bf16),
        scratch_shapes=[pltpu.VMEM((S, D), bf16), pltpu.VMEM((S + 2 * PAD, D), bf16), pltpu.VMEM((S, DH), bf16),
                        pltpu.VMEM((DH, S), bf16), pltpu.VMEM((nb * D, tq), bf16), pltpu.VMEM((nb * D, tq), bf16),
                        pltpu.VMEM((S, tq), f32), pltpu.VMEM((S, tq), f32), pltpu.VMEM((16, tq), f32), pltpu.VMEM((len(vpu) + 1, DH, VK, 128), f32), pltpu.VMEM((DH, 8, tq), f32), pltpu.VMEM((DH, 8, tq), f32),
                        pltpu.VMEM((D, D), bf16), pltpu.VMEM((D + 2 * DH, D), bf16)]
                       + [pltpu.VMEM(a.shape, bf16) for a in hin[4:]] + [pltpu.SemaphoreType.DMA((nb + 8,))],
        compiler_params=pltpu.CompilerParams(dimension_semantics=("arbitrary",), vmem_limit_bytes=100 * 1024 * 1024),
    )(*hin)
    return out.reshape(1, S, D)


@jax.jit
def pallas_recurrent_scan__grouped_kv_mqa__mixer_s_mlp__prompt_kernel(
        A_x, A_wq, A_wk, A_wv, A_wo, B_x, B_w1, B_w2, B_w3, B_w4):
    return _run(A_x, A_wq, A_wk, A_wv, A_wo, B_x, B_w1, B_w2, B_w3, B_w4)
```
